```python
import jax
import jax.numpy as jnp

def _softmax(x, axis=-1):
    return jax.nn.softmax(x, axis=axis)
def _gelu(x):
    return jax.nn.gelu(x, approximate=True)
def _silu(x):
    return jax.nn.silu(x)
def _sigmoid(x):
    return jax.nn.sigmoid(x)
def _layernorm(x, axis=-1, eps=1e-5):
    m = jnp.mean(x, axis=axis, keepdims=True)
    v = jnp.var(x, axis=axis, keepdims=True)
    return (x - m) / jnp.sqrt(v + eps)
def _scatter_add(tgt, idx, src, axis=0):
    return tgt.at[idx].add(src)
def _segment_sum(src, seg, n):
    return jax.ops.segment_sum(src, seg, n)
class _Rng:
    def __init__(self, key):
        self._k = key
    def _next(self):
        self._k, sub = jax.random.split(self._k)
        return sub
    def normal(self, shape):
        return jax.random.normal(self._next(), shape, dtype=jnp.bfloat16)
    def randint(self, lo, hi, shape):
        return jax.random.randint(self._next(), shape, lo, hi, dtype=jnp.int32)
    def uniform(self, shape, lo=0.0, hi=1.0):
        return jax.random.uniform(self._next(), shape, jnp.bfloat16, lo, hi)
    def permutation(self, n):
        return jax.random.permutation(self._next(), n)


kernel_name = 'standalone__gqa_block_cached__near_ridge'

def setup_inputs():
    _rng = _Rng(jax.random.key(int.from_bytes(__import__("os").urandom(4), "little")))
    _w = (lambda a: (lambda t: t.astype(jnp.bfloat16) if jnp.issubdtype(t.dtype, jnp.floating) else t)(jnp.asarray(a)))
    B, Sq, D = 16, 240, 640
    Hq, Hkv, Sk, Dh = 32, 32, 1024, 128
    assert Hq % Hkv == 0, (Hq, Hkv)
    return {
        "x": _w((lambda *s: _rng.normal(s) * 0.05)(B, Sq, D)),
        "k_cache": _w((lambda *s: _rng.normal(s) * 0.05)(B, Hkv, Sk, Dh)),
        "v_cache": _w((lambda *s: _rng.normal(s) * 0.05)(B, Hkv, Sk, Dh)),
        "wq": _w((lambda *s: _rng.normal(s) * 0.05)(D, Hq * Dh) * (D ** -0.5)),
        "wo": _w((lambda *s: _rng.normal(s) * 0.05)(Hq * Dh, D) * ((Hq * Dh) ** -0.5)),
    }

def reference(x, k_cache, v_cache, wq, wo):
    B, Sq, D = x.shape
    Hq, Dh = 32, 128
    Hkv = k_cache.shape[1]
    rep = Hq // Hkv
    q = (lambda x, *d: x.transpose(*d))((x @ wq).reshape(B, Sq, Hq, Dh), 0, 2, 1, 3)
    k = jnp.repeat(k_cache, rep, axis=1)
    v = jnp.repeat(v_cache, rep, axis=1)
    scores = jnp.einsum("bhqd,bhkd->bhqk", q, k) * (Dh ** -0.5)
    p = _softmax(scores, axis=-1)
    o = jnp.einsum("bhqk,bhkd->bhqd", p, v)
    return (lambda x, *d: x.transpose(*d))(o, 0, 2, 1, 3).reshape(B, Sq, Hq * Dh) @ wo
```

```python
import functools, math
import jax, jax.numpy as jnp
from jax.experimental import pallas as pl
from jax.experimental.pallas import tpu as pltpu

LOG2E = 1.4426950408889634
S8 = 'R0 q0 q1 A0 q2 A1 q3 C0 A2 R1 C1 A3 q4 C2 A4 q5 C3 A5 q6 C4 A6 q7 p00 C5 A7 p01 C6 p02 C7 p03 p04 p10 p11 p12 p13 p14'

def make(HB=8, sched=S8, flags=None, pin=0, div=1):
    Dh = 128; H = 32; B = 16
    NG = H // HB; W = HB * Dh; nj = HB // 4; NSTEP = B * NG // div
    def kern(x_hbm, k_hbm, v_hbm, wq_hbm, wo_hbm, o_hbm,
             xbuf, kbuf, vbuf, wq_ref, wo_ref, acc_ref, obuf, wsem, ksem, vsem, xsem, osem):
        c = (Dh ** -0.5) * LOG2E
        def wqcopy(i):
            return pltpu.make_async_copy(wq_hbm.at[:, pl.ds(pl.multiple_of(i * W, W), W)], wq_ref.at[i], wsem.at[0, i])
        def wocopy(i):
            return pltpu.make_async_copy(wo_hbm.at[pl.ds(pl.multiple_of(i * W, W), W), :], wo_ref.at[i], wsem.at[1, i])
        def kcopy(t):
            return pltpu.make_async_copy(k_hbm.at[pl.ds(t * HB, HB)], kbuf.at[t & 1], ksem.at[t & 1])
        def vcopy(t):
            return pltpu.make_async_copy(v_hbm.at[pl.ds(t * HB, HB)], vbuf.at[t & 1], vsem.at[t & 1])
        def xcopy(bb):
            return pltpu.make_async_copy(x_hbm.at[bb], xbuf.at[bb & 1], xsem.at[bb & 1])
        def ocopy(bb):
            return pltpu.make_async_copy(obuf.at[bb & 1], o_hbm.at[bb], osem.at[bb & 1])
        xcopy(0).start(); wqcopy(0).start()
        kcopy(0).start(); vcopy(0).start(); wocopy(0).start()
        acc_ref[...] = jnp.zeros_like(acc_ref)

        def step(s, carry):
            b = s >> (NG.bit_length() - 1)
            g = s & (NG - 1)
            slot = s & 1
            xs = b & 1
            @pl.when(s + 1 < NSTEP)
            def _():
                kcopy(s + 1).start(); vcopy(s + 1).start()
            @pl.when(s < NG)
            def _():
                @pl.when(s + 1 < NG)
                def _():
                    wqcopy(s + 1).start(); wocopy(s + 1).start()
                wqcopy(s).wait(); wocopy(s).wait()
            @pl.when(g == 0)
            def _():
                @pl.when(b + 1 < B // div)
                def _(): xcopy(b + 1).start()
                @pl.when(b > 0)
                def _(): ocopy(b - 1).start()
                @pl.when(b > 1)
                def _(): ocopy(b - 2).wait()
                xcopy(b).wait()
            kcopy(s).wait(); vcopy(s).wait()

            RR = {}; OO = {}; S = {}; O = {}; q = {}
            def Rm(j):
                RR[j] = jnp.dot(xbuf[xs, :, 512:], wq_ref[g, 512:, j*512:(j+1)*512], preferred_element_type=jnp.float32)
            def qq(h):
                j, i = divmod(h, 4)
                r = jnp.dot(xbuf[xs, :, :512], wq_ref[g, :512, h*128:(h+1)*128], preferred_element_type=jnp.float32)
                q[h] = ((r + RR[j][:, i*128:(i+1)*128]) * c).astype(jnp.bfloat16)
            def A(h):
                S[h] = jax.lax.dot_general(q.pop(h), kbuf[slot, h], (((1,),(1,)),((),())), preferred_element_type=jnp.float32)
            def C(h):
                sc = S.pop(h)
                m = jnp.max(sc, axis=-1, keepdims=True)
                p = jnp.exp2(sc - m)
                if pin:
                    t = [p[:, i*128:(i+1)*128] for i in range(8)]
                    p1 = (t[0] + t[1]) + (t[2] + t[3])
                    p2 = (t[4] + t[5]) + (t[6] + t[7])
                    ps = p1 + p2
                    p = jnp.concatenate(t[:3] + [jnp.minimum(t[3], p1)] + t[4:7] + [jnp.minimum(t[7], ps)], axis=-1)
                    l = jnp.sum(ps, axis=-1, keepdims=True)
                else:
                    l = jnp.sum(p, axis=-1, keepdims=True)
                r = pl.reciprocal(l, approx=True)
                r = r * (2.0 - l * r)
                o = jnp.dot(p.astype(jnp.bfloat16), vbuf[slot, h], preferred_element_type=jnp.float32)
                O[h] = o * r
            def pp(u):
                j, n = divmod(u, 10)
                if j not in OO:
                    OO[j] = jnp.concatenate([O.pop(4*j+i) for i in range(4)], axis=-1).astype(jnp.bfloat16)
                y = jnp.dot(OO[j], wo_ref[g, j*512:(j+1)*512, n*128:(n+1)*128], preferred_element_type=jnp.float32)
                a = acc_ref[:, n*128:(n+1)*128]
                if j == 0: a = jnp.where(g == 0, 0.0, a)
                a = a + y
                acc_ref[:, n*128:(n+1)*128] = a
                if j == nj - 1:
                    obuf[xs, :, n*128:(n+1)*128] = a.astype(obuf.dtype)
            for t in sched.split():
                {"A": A, "C": C, "R": Rm, "q": qq, "p": pp}[t[0]](int(t[1:]))
            return carry
        jax.lax.fori_loop(0, NSTEP, step, 0)
        bl = B // div - 1
        ocopy(bl).start(); ocopy(bl - 1).wait(); ocopy(bl).wait()

    def fn(x, k_cache, v_cache, wq, wo):
        _, Sq, D = x.shape
        Sk = k_cache.shape[2]
        bf = jnp.bfloat16
        anyspec = pl.BlockSpec(memory_space=pl.ANY)
        return pl.pallas_call(
            kern,
            in_specs=[anyspec] * 5, out_specs=anyspec,
            out_shape=jax.ShapeDtypeStruct((B, Sq, D), x.dtype),
            scratch_shapes=[pltpu.VMEM((2, Sq, D), bf), pltpu.VMEM((2, HB, Sk, Dh), bf), pltpu.VMEM((2, HB, Sk, Dh), bf),
                            pltpu.VMEM((NG, D, W), bf), pltpu.VMEM((NG, W, D), bf),
                            pltpu.VMEM((Sq, D), jnp.float32), pltpu.VMEM((2, Sq, D), bf),
                            pltpu.SemaphoreType.DMA((2, NG)), pltpu.SemaphoreType.DMA((2,)), pltpu.SemaphoreType.DMA((2,)),
                            pltpu.SemaphoreType.DMA((2,)), pltpu.SemaphoreType.DMA((2,))],
            compiler_params=pltpu.CompilerParams(vmem_limit_bytes=100 * 1024 * 1024, flags=flags, disable_bounds_checks=True),
            name="gqa",
        )(x, k_cache.reshape(B * H, Sk, Dh), v_cache.reshape(B * H, Sk, Dh), wq, wo)
    return fn


@jax.jit
def pallas_standalone__gqa_block_cached__near_ridge_kernel(x, k_cache, v_cache, wq, wo):
    return make(**dict())(x, k_cache, v_cache, wq, wo)
```

```python
import functools, math
import jax, jax.numpy as jnp
from jax.experimental import pallas as pl
from jax.experimental.pallas import tpu as pltpu

LOG2E = 1.4426950408889634

def gen(mid, H=32):
    out = "R0 q0 A0 q1 A1 q2 q3 R1 C0 A2 q4 C1 A3 q5 C2 A4 q6 C3 q7".split()
    nj = H // 4
    for j in range(1, nj):
        last = j == nj - 1
        for t in (mid if not last else "A1 C0 p0 A2 p1 C1 A3 C2 p2 C3 p3 p4").split():
            k, i = t[0], int(t[1:])
            if k in "AC": out.append(f"{k}{4*j+i}")
            elif k == "q": out.append(f"q{4*(j+1)+i}")
            elif k == "R": out.append(f"R{j+1}")
            elif k == "p": out.append(f"p{(j-1)*10+i}")
    out += [f"p{(nj-1)*10+i}" for i in range(5)]
    return " ".join(out)

MID = "A1 R0 C0 p0 A2 p1 C1 p2 q0 A3 p3 C2 q1 A4 p4 C3 q2 q3"

def make(mid=MID, sched=None, flags=None, pin=1, NS=4, H=32, B=16, WD=1):
    Dh = 128
    nj = H // 4
    sched_ = sched or gen(mid, H)
    fl = {"XLA_TPU_RESCHEDULE_DMA_DONES": True}
    fl.update(flags or {})
    def kern(x_hbm, k_hbm, v_hbm, wq_hbm, wo_hbm, o_hbm,
             xbuf, kbuf, vbuf, wq_ref, wo_ref, acc_ref, obuf, qsem, wsem, ksem, vsem, xsem, osem):
        c = (Dh ** -0.5) * LOG2E
        def wqcopy(j):
            return pltpu.make_async_copy(wq_hbm.at[:, pl.ds(j * 512, 512)], wq_ref.at[j], qsem.at[j])
        def wocopy(j):
            return pltpu.make_async_copy(wo_hbm.at[pl.ds(j * 512, 512), :], wo_ref.at[j], wsem.at[j])
        def kcopy(b, t):
            return pltpu.make_async_copy(k_hbm.at[b * 32 + t], kbuf.at[t % NS], ksem.at[t % NS])
        def vcopy(b, t):
            return pltpu.make_async_copy(v_hbm.at[b * 32 + t], vbuf.at[t % NS], vsem.at[t % NS])
        def xcopy(bb):
            return pltpu.make_async_copy(x_hbm.at[bb], xbuf.at[bb & 1], xsem.at[bb & 1])
        def ocopy(bb):
            return pltpu.make_async_copy(obuf.at[bb & 1], o_hbm.at[bb], osem.at[bb & 1])
        xcopy(0).start(); wqcopy(0).start(); kcopy(0, 0).start()
        for j in range(1, WD + 1): wqcopy(j).start()
        vcopy(0, 0).start()
        for t in range(1, NS):
            kcopy(0, t).start(); vcopy(0, t).start()

        def step(b, carry):
            xs = b & 1
            first = b == 0
            more = b + 1 < B
            @pl.when(more)
            def _(): xcopy(b + 1).start()
            @pl.when(b > 0)
            def _(): ocopy(b - 1).start()
            @pl.when(b > 1)
            def _(): ocopy(b - 2).wait()
            xcopy(b).wait()
            RR = {}; OO = {}; S = {}; O = {}; q = {}
            def prefetch(cp, h):
                t = h + NS
                if t < H: cp(b, t).start()
                else:
                    @pl.when(more)
                    def _(): cp(b + 1, t - H).start()
            def Rm(j):
                @pl.when(first)
                def _():
                    wqcopy(j).wait()
                    if j + WD + 1 < nj: wqcopy(j + WD + 1).start()
                    wocopy(j).start()
                RR[j] = jnp.dot(xbuf[xs, :, 512:], wq_ref[j, 512:, :], preferred_element_type=jnp.float32)
            def qq(h):
                j, i = divmod(h, 4)
                r = jnp.dot(xbuf[xs, :, :512], wq_ref[j, :512, i*128:(i+1)*128], preferred_element_type=jnp.float32)
                q[h] = ((r + RR[j][:, i*128:(i+1)*128]) * c).astype(jnp.bfloat16)
            def A(h):
                kcopy(b, h).wait()
                S[h] = jax.lax.dot_general(q.pop(h), kbuf[h % NS], (((1,),(1,)),((),())), preferred_element_type=jnp.float32)
                prefetch(kcopy, h)
            def C(h):
                sc = S.pop(h)
                m = jnp.max(sc, axis=-1, keepdims=True)
                p = jnp.exp2(sc - m)
                if pin:
                    t = [p[:, i*128:(i+1)*128] for i in range(8)]
                    p1 = (t[0] + t[1]) + (t[2] + t[3])
                    p2 = (t[4] + t[5]) + (t[6] + t[7])
                    ps = p1 + p2
                    p = jnp.concatenate(t[:3] + [jnp.minimum(t[3], p1)] + t[4:7] + [jnp.minimum(t[7], ps)], axis=-1)
                    l = jnp.sum(ps, axis=-1, keepdims=True)
                else:
                    l = jnp.sum(p, axis=-1, keepdims=True)
                r = pl.reciprocal(l, approx=True)
                r = r * (2.0 - l * r)
                vcopy(b, h).wait()
                o = jnp.dot(p.astype(jnp.bfloat16), vbuf[h % NS], preferred_element_type=jnp.float32)
                prefetch(vcopy, h)
                O[h] = o * r
            def pp(u):
                j, n = divmod(u, 10)
                if j not in OO:
                    @pl.when(first)
                    def _(): wocopy(j).wait()
                    OO[j] = jnp.concatenate([O.pop(4*j+i) for i in range(4)], axis=-1).astype(jnp.bfloat16)
                a = jnp.dot(OO[j], wo_ref[j, :, n*128:(n+1)*128], preferred_element_type=jnp.float32)
                if j > 0: a = a + acc_ref[:, n*128:(n+1)*128]
                if j < nj - 1: acc_ref[:, n*128:(n+1)*128] = a
                else: obuf[xs, :, n*128:(n+1)*128] = a.astype(obuf.dtype)
            for t in sched_.split():
                {"A": A, "C": C, "R": Rm, "q": qq, "p": pp}[t[0]](int(t[1:]))
            return carry
        jax.lax.fori_loop(0, B, step, 0)
        ocopy(B - 1).start(); ocopy(B - 2).wait(); ocopy(B - 1).wait()

    def fn(x, k_cache, v_cache, wq, wo):
        B_, Sq, D = x.shape
        Sk = k_cache.shape[2]
        bf = jnp.bfloat16
        anyspec = pl.BlockSpec(memory_space=pl.ANY)
        return pl.pallas_call(
            kern,
            in_specs=[anyspec] * 5, out_specs=anyspec,
            out_shape=jax.ShapeDtypeStruct((B_, Sq, D), x.dtype),
            scratch_shapes=[pltpu.VMEM((2, Sq, D), bf), pltpu.VMEM((NS, Sk, Dh), bf), pltpu.VMEM((NS, Sk, Dh), bf),
                            pltpu.VMEM((nj, D, 512), bf), pltpu.VMEM((nj, 512, D), bf),
                            pltpu.VMEM((Sq, D), jnp.float32), pltpu.VMEM((2, Sq, D), bf),
                            pltpu.SemaphoreType.DMA((nj,)), pltpu.SemaphoreType.DMA((nj,)),
                            pltpu.SemaphoreType.DMA((NS,)), pltpu.SemaphoreType.DMA((NS,)),
                            pltpu.SemaphoreType.DMA((2,)), pltpu.SemaphoreType.DMA((2,))],
            compiler_params=pltpu.CompilerParams(vmem_limit_bytes=100 * 1024 * 1024, flags=fl, disable_bounds_checks=True),
            name="gqa",
        )(x, k_cache.reshape(B_ * 32, Sk, Dh), v_cache.reshape(B_ * 32, Sk, Dh), wq, wo)
    return fn


@jax.jit
def pallas_standalone__gqa_block_cached__near_ridge_kernel(x, k_cache, v_cache, wq, wo):
    return make(**dict())(x, k_cache, v_cache, wq, wo)
```

```python
import jax
import jax.numpy as jnp
from jax.experimental import pallas as pl
from jax.experimental.pallas import tpu as pltpu

LOG2E = 1.4426950408889634
H = 32
DH = 128
NS = 4
NJ = H // 4

SCHEDULE = (
    "R0 q0 A0 q1 A1 q2 q3 R1 C0 A2 q4 C1 A3 q5 C2 A4 q6 C3 q7 A5 R2 C4 p0 q8 A6 q9 C5 p1 "
    "A7 p2 C6 q10 A8 q11 C7 p3 p4 A9 C8 R3 p10 q12 p11 A10 C9 q13 A11 q14 p12 C10 A12 q15 "
    "C11 A13 p13 p14 R4 C12 p20 q16 q17 A14 C13 p21 A15 p22 C14 q18 q19 A16 C15 p23 R5 "
    "p24 A17 C16 p30 q20 A18 q21 C17 p31 A19 p32 C18 q23 q22 A20 C19 p33 R6 p34 A21 C20 "
    "p40 q24 A22 q25 C21 p41 A23 p42 C22 q26 p44 A24 C23 p43 R7 q27 A25 C24 p50 q28 A26 "
    "q29 C25 p51 A27 p52 C26 q31 q30 A28 C27 p53 p54 A29 C28 p61 p60 A30 C29 A31 C30 p63 "
    "C31 p64 p62 p71 p70 p72 p73 p74 "
).split()


def _kernel(x_hbm, k_hbm, v_hbm, wq_hbm, wo_hbm, o_hbm,
            xbuf, kbuf, vbuf, wq_ref, wo_ref, acc_ref, obuf,
            qsem, wsem, ksem, vsem, xsem, osem):
    nb = x_hbm.shape[0]
    sk = kbuf.shape[1]
    scale = (DH ** -0.5) * LOG2E

    def wq_copy(j):
        return pltpu.make_async_copy(wq_hbm.at[:, pl.ds(j * 512, 512)], wq_ref.at[j], qsem.at[j])

    def wo_copy(j):
        return pltpu.make_async_copy(wo_hbm.at[pl.ds(j * 512, 512), :], wo_ref.at[j], wsem.at[j])

    def k_copy(b, h):
        return pltpu.make_async_copy(k_hbm.at[b * H + h], kbuf.at[h % NS], ksem.at[h % NS])

    def v_copy(b, h):
        return pltpu.make_async_copy(v_hbm.at[b * H + h], vbuf.at[h % NS], vsem.at[h % NS])

    def x_copy(b):
        return pltpu.make_async_copy(x_hbm.at[b], xbuf.at[b & 1], xsem.at[b & 1])

    def o_copy(b):
        return pltpu.make_async_copy(obuf.at[b & 1], o_hbm.at[b], osem.at[b & 1])

    x_copy(0).start()
    wq_copy(0).start()
    for h in range(NS):
        k_copy(0, h).start()
        v_copy(0, h).start()

    def step(b, carry):
        slot = b & 1
        first = b == 0
        more = b + 1 < nb

        @pl.when(more)
        def _():
            x_copy(b + 1).start()

        @pl.when(b > 0)
        def _():
            o_copy(b - 1).start()

        @pl.when(b > 1)
        def _():
            o_copy(b - 2).wait()

        x_copy(b).wait()

        q_tail, q, scores, o, o4 = {}, {}, {}, {}, {}

        def refill(copy, h):
            if h + NS < H:
                copy(b, h + NS).start()
            else:
                @pl.when(more)
                def _():
                    copy(b + 1, h + NS - H).start()

        def q_proj_tail(j):
            @pl.when(first)
            def _():
                wq_copy(j).wait()
                if j + 1 < NJ:
                    wq_copy(j + 1).start()
                wo_copy(j).start()

            q_tail[j] = jnp.dot(xbuf[slot, :, 512:], wq_ref[j, 512:, :],
                                preferred_element_type=jnp.float32)

        def q_proj(h):
            j, i = divmod(h, 4)
            cols = slice(i * DH, (i + 1) * DH)
            r = jnp.dot(xbuf[slot, :, :512], wq_ref[j, :512, cols],
                        preferred_element_type=jnp.float32)
            q[h] = ((r + q_tail[j][:, cols]) * scale).astype(jnp.bfloat16)

        def qk(h):
            k_copy(b, h).wait()
            scores[h] = jax.lax.dot_general(
                q.pop(h), kbuf[h % NS], (((1,), (1,)), ((), ())),
                preferred_element_type=jnp.float32)
            refill(k_copy, h)

        def softmax_pv(h):
            s = scores.pop(h)
            p = jnp.exp2(s - jnp.max(s, axis=-1, keepdims=True))
            t = [p[:, i * 128:(i + 1) * 128] for i in range(sk // 128)]
            lo = (t[0] + t[1]) + (t[2] + t[3])
            tot = lo + ((t[4] + t[5]) + (t[6] + t[7]))
            p = jnp.concatenate(
                t[:3] + [jnp.minimum(t[3], lo)] + t[4:7] + [jnp.minimum(t[7], tot)], axis=-1)
            l = jnp.sum(tot, axis=-1, keepdims=True)
            r = pl.reciprocal(l, approx=True)
            r = r * (2.0 - l * r)
            v_copy(b, h).wait()
            pv = jnp.dot(p.astype(jnp.bfloat16), vbuf[h % NS],
                         preferred_element_type=jnp.float32)
            refill(v_copy, h)
            o[h] = pv * r

        def o_proj(u):
            j, n = divmod(u, 10)
            cols = slice(n * 128, (n + 1) * 128)
            if j not in o4:
                @pl.when(first)
                def _():
                    wo_copy(j).wait()

                o4[j] = jnp.concatenate(
                    [o.pop(4 * j + i) for i in range(4)], axis=-1).astype(jnp.bfloat16)
            y = jnp.dot(o4[j], wo_ref[j, :, cols], preferred_element_type=jnp.float32)
            if j > 0:
                y = y + acc_ref[:, cols]
            if j < NJ - 1:
                acc_ref[:, cols] = y
            else:
                obuf[slot, :, cols] = y.astype(obuf.dtype)

        units = {"R": q_proj_tail, "q": q_proj, "A": qk, "C": softmax_pv, "p": o_proj}
        for unit in SCHEDULE:
            units[unit[0]](int(unit[1:]))
        return carry

    jax.lax.fori_loop(0, nb, step, 0)
    o_copy(nb - 1).start()
    o_copy(nb - 2).wait()
    o_copy(nb - 1).wait()


@jax.jit
def pallas_standalone__gqa_block_cached__near_ridge_kernel(x, k_cache, v_cache, wq, wo):
    B, Sq, D = x.shape
    _, Hkv, Sk, Dh = k_cache.shape
    assert (Hkv, Sk, Dh, D) == (H, 1024, DH, 640) and B >= 2
    bf16 = jnp.bfloat16
    hbm = pl.BlockSpec(memory_space=pl.ANY)
    return pl.pallas_call(
        _kernel,
        in_specs=[hbm] * 5,
        out_specs=hbm,
        out_shape=jax.ShapeDtypeStruct((B, Sq, D), x.dtype),
        scratch_shapes=[
            pltpu.VMEM((2, Sq, D), bf16),
            pltpu.VMEM((NS, Sk, Dh), bf16),
            pltpu.VMEM((NS, Sk, Dh), bf16),
            pltpu.VMEM((NJ, D, 512), bf16),
            pltpu.VMEM((NJ, 512, D), bf16),
            pltpu.VMEM((Sq, D), jnp.float32),
            pltpu.VMEM((2, Sq, D), x.dtype),
            pltpu.SemaphoreType.DMA((NJ,)),
            pltpu.SemaphoreType.DMA((NJ,)),
            pltpu.SemaphoreType.DMA((NS,)),
            pltpu.SemaphoreType.DMA((NS,)),
            pltpu.SemaphoreType.DMA((2,)),
            pltpu.SemaphoreType.DMA((2,)),
        ],
        compiler_params=pltpu.CompilerParams(
            vmem_limit_bytes=100 * 1024 * 1024,
            disable_bounds_checks=True,
            flags={"XLA_TPU_RESCHEDULE_DMA_DONES": True},
        ),
        name="gqa",
    )(x, k_cache.reshape(B * H, Sk, Dh), v_cache.reshape(B * H, Sk, Dh), wq, wo)
```
